```python
import jax
import jax.numpy as jnp

def _softmax(x, axis=-1):
    return jax.nn.softmax(x, axis=axis)
def _gelu(x):
    return jax.nn.gelu(x, approximate=True)
def _silu(x):
    return jax.nn.silu(x)
def _sigmoid(x):
    return jax.nn.sigmoid(x)
def _layernorm(x, axis=-1, eps=1e-5):
    m = jnp.mean(x, axis=axis, keepdims=True)
    v = jnp.var(x, axis=axis, keepdims=True)
    return (x - m) / jnp.sqrt(v + eps)
def _scatter_add(tgt, idx, src, axis=0):
    return tgt.at[idx].add(src)
def _segment_sum(src, seg, n):
    return jax.ops.segment_sum(src, seg, n)
class _Rng:
    def __init__(self, key):
        self._k = key
    def _next(self):
        self._k, sub = jax.random.split(self._k)
        return sub
    def normal(self, shape):
        return jax.random.normal(self._next(), shape, dtype=jnp.bfloat16)
    def randint(self, lo, hi, shape):
        return jax.random.randint(self._next(), shape, lo, hi, dtype=jnp.int32)
    def uniform(self, shape, lo=0.0, hi=1.0):
        return jax.random.uniform(self._next(), shape, jnp.bfloat16, lo, hi)
    def permutation(self, n):
        return jax.random.permutation(self._next(), n)


kernel_name = 'recurrent_scan__ssm_conv_h3__mixer_token_mlp__prompt'

def setup_inputs():
    _rng = _Rng(jax.random.key(int.from_bytes(__import__("os").urandom(4), "little")))
    _w = (lambda a: (lambda t: t.astype(jnp.bfloat16) if jnp.issubdtype(t.dtype, jnp.floating) else t)(jnp.asarray(a)))
    def _A_setup():
        B, S, D = 1, 2048, 576
        ks = 4
        return {
            "q": _w((lambda *s: _rng.normal(s) * 0.05)(B, S, D)),
            "k": _w((lambda *s: _rng.normal(s) * 0.05)(B, S, D)),
            "v": _w((lambda *s: _rng.normal(s) * 0.05)(B, S, D)),
            "shift_k": _w((lambda *s: _rng.normal(s) * 0.05)(D, ks) * 0.5),
            "ssm_k": _w((lambda *s: _rng.normal(s) * 0.05)(D, S) * (1.0 / S ** 0.5)),
            "ssm_D": _w((lambda *s: _rng.normal(s) * 0.05)(D)),
        }
    _A_in = _A_setup()

    def _B_setup():
        B, S, D, F = 1, 2048, 576, 4608
        return {
            "x": _w((lambda *s: _rng.normal(s) * 0.05)(B, S, D)),
            "w1": _w((lambda *s: _rng.normal(s) * 0.05)(S, F) * (S ** -0.5)),
            "b1": _w((lambda *s: _rng.normal(s) * 0.05)(F) * 0.02),
            "w2": _w((lambda *s: _rng.normal(s) * 0.05)(F, S) * (F ** -0.5)),
            "b2": _w((lambda *s: _rng.normal(s) * 0.05)(S) * 0.02),
        }
    _B_in = _B_setup()

    return {
        "A_q": _A_in["q"],
        "A_k": _A_in["k"],
        "A_v": _A_in["v"],
        "A_shift_k": _A_in["shift_k"],
        "A_ssm_k": _A_in["ssm_k"],
        "A_ssm_D": _A_in["ssm_D"],
        "B_x": _B_in["x"],
        "B_w1": _B_in["w1"],
        "B_b1": _B_in["b1"],
        "B_w2": _B_in["w2"],
        "B_b2": _B_in["b2"],
    }

def reference(A_q, A_k, A_v, A_shift_k, A_ssm_k, A_ssm_D, B_x, B_w1, B_b1, B_w2, B_b2):
    def _A_ref(q, k, v, shift_k, ssm_k, ssm_D):
        B, S, D = q.shape
        ks = shift_k.shape[-1]
        k_pad = jnp.pad(k, ((0, 0), (ks - 1, 0), (0, 0)))
        k_shift = jnp.zeros_like(k)
        for t in range(ks):
            k_shift = k_shift + k_pad[:, t:t + S, :] * shift_k[:, ks - 1 - t][None, None, :]
        kv = k_shift * v
        L = 2 * S
        kv_pad = jnp.pad(kv, ((0, 0), (0, S), (0, 0)))
        kf_pad = jnp.pad(ssm_k, ((0, 0), (0, S)))
        kv_f = (lambda x, axes=(-2,-1): jnp.fft.rfft2(x.astype(jnp.float32), axes=axes))(kv_pad[:, None, :, :], axes=(1, 2))
        kf_f = (lambda x, axes=(-2,-1): jnp.fft.rfft2(x.astype(jnp.float32), axes=axes))(kf_pad[:, None, :], axes=(1, 2))
        kf_f = (lambda x, *d: x.transpose(*d))(kf_f, 1, 2, 0)
        y_f = kv_f * kf_f[None, :, :, :]
        y = (lambda x, s, axes=(-2,-1): jnp.fft.irfft2(x, s=s, axes=axes).astype(jnp.bfloat16))(y_f, (1, L), axes=(1, 2))[:, 0, :S, :]
        y = y + kv * ssm_D[None, None, :]
        return q * y

    def _B_ref(x, w1, b1, w2, b2):
        B, S, D = x.shape
        h = _layernorm(x, axis=-1)
        u = jnp.einsum("bsd,sf->bdf", h, w1) + b1
        u = _gelu(u)
        y = jnp.einsum("bdf,fs->bds", u, w2) + b2
        return (lambda x, *d: x.transpose(*d))(y, 0, 2, 1)

    x = A_q
    xn = _layernorm(x, axis=-1)
    s = _A_ref(xn, A_k, A_v, A_shift_k, A_ssm_k, A_ssm_D)
    g = _silu(_B_ref(xn, B_w1, B_b1, B_w2, B_b2))
    return x + s * g
```

```python
import numpy as np
import ml_dtypes
import jax
import jax.numpy as jnp
from jax import lax
import jax.experimental.pallas as pl
import jax.experimental.pallas.tpu as pltpu

S, D, F = 2048, 576, 4608
KS = 4
TF = 768
NF = F // TF
BL = 128
J = S // BL
KC = 512
NKC = S // KC
CC = D // (NF - 2)
EPS = 1e-5
BF = jnp.bfloat16
F32 = jnp.float32

_n = np.arange(BL)[None, :]
_f = np.arange(BL)[:, None]
_th = np.pi * (2 * _f + 1) * _n / (2 * BL)
_FT = np.concatenate([np.cos(_th), -np.sin(_th)], 0)
FM_NP = np.ascontiguousarray(_FT.T).astype(ml_dtypes.bfloat16)
FI_NP = (_FT / BL).astype(ml_dtypes.bfloat16)


def _gelu(x):
    return 0.5 * x * (1.0 + jnp.tanh(0.7978845608028654 * (x + 0.044715 * (x * x * x))))


def _dot(a, b):
    return jnp.dot(a, b, preferred_element_type=F32)


def build(cfg):
    LNC = cfg.get("LNC", 128)
    MR = cfg.get("MR", 16)
    N1 = cfg.get("N1", 768)
    N2 = cfg.get("N2", 512)
    PR = cfg.get("PR", 48)
    debug = cfg.get("debug", False)
    order = cfg.get("order", "fwd,mm1,mac,mm2,inv")

    def kernel(q_hbm, k_hbm, v_hbm, f_hbm, w1_hbm, w2_hbm, sk_ref, d_ref, b1_ref, b2_ref, fm_ref, fi_ref,
               o_hbm,
               xT, xnT, hT, kT, vT, fT, sT, w1buf, w2buf, acc, uacc, ubf,
               kvb, Xs, Gs, Ys, taps, tpad, obuf,
               sem_q, sem_w10, sem_w1, sem_w2, sem_kvf, sem_o):

        def cp_q(i):
            return pltpu.make_async_copy(q_hbm.at[:, pl.ds(i * KC, KC)], xT.at[:, pl.ds(i * KC, KC)], sem_q.at[i])

        def cp_w10(i):
            return pltpu.make_async_copy(w1_hbm.at[pl.ds(i * KC, KC), pl.ds(0, TF)],
                                         w1buf.at[0, pl.ds(i * KC, KC), :], sem_w10.at[i])

        def cp_w1(t, slot):
            return pltpu.make_async_copy(w1_hbm.at[:, pl.ds(pl.multiple_of(t * TF, TF), TF)], w1buf.at[slot], sem_w1.at[slot])

        def cp_w2(t, slot):
            return pltpu.make_async_copy(w2_hbm.at[pl.ds(pl.multiple_of(t * TF, TF), TF), :], w2buf.at[slot], sem_w2.at[slot])

        def cp_kvf(c):
            rows = pl.ds(pl.multiple_of(c * CC, 16), CC)
            return [pltpu.make_async_copy(src.at[rows, :], dst.at[rows, :], sem_kvf.at[a, c % 2])
                    for a, (src, dst) in enumerate(((k_hbm, kT), (v_hbm, vT), (f_hbm, fT)))]

        def cp_o(i):
            return pltpu.make_async_copy(obuf.at[:, pl.ds(i * KC, KC)], o_hbm.at[:, pl.ds(i * KC, KC)], sem_o.at[i])

        for i in range(NKC):
            cp_q(i).start()
            cp_w10(i).start()
        cp_w2(0, 0).start()
        cp_w1(1, 1).start()
        for c in cp_kvf(0):
            c.start()
        cp_w2(1, 1).start()

        tpad[...] = jnp.zeros_like(tpad)
        tpad[0:KS, 0:D] = sk_ref[...].astype(F32)
        tpad[KS:KS + 1, 0:D] = d_ref[...].astype(F32).reshape(1, D)
        for ct in range(5):
            taps[ct * 128:(ct + 1) * 128, :] = tpad[:, ct * 128:(ct + 1) * 128].T

        lane = lax.broadcasted_iota(jnp.int32, (8, 128), 1)
        sgn8 = (1 - 2 * (lane & 1)).astype(F32)

        def ln_cols(c0):
            cols = pl.ds(c0, LNC)
            x = xT[:, cols].astype(F32)
            m = jnp.sum(x, axis=0, keepdims=True) * (1.0 / D)
            xc = x - m
            var = jnp.sum(xc * xc, axis=0, keepdims=True) * (1.0 / D)
            xn = (xc * lax.rsqrt(var + EPS)).astype(BF)
            xnT[:, cols] = xn
            xf = xn.astype(F32)
            m2 = jnp.sum(xf, axis=0, keepdims=True) * (1.0 / D)
            xc2 = xf - m2
            var2 = jnp.sum(xc2 * xc2, axis=0, keepdims=True) * (1.0 / D)
            hT[:, cols] = (xc2 * lax.rsqrt(var2 + EPS)).astype(BF)

        def ln_chunk(i):
            for r in range(KC // LNC):
                ln_cols(i * KC + r * LNC)

        def mm1(slot, b1row):
            for n in range(TF // N1):
                u = _dot(hT[...], w1buf[slot, :, n * N1:(n + 1) * N1])
                ubf[:, n * N1:(n + 1) * N1] = _gelu(u + b1row[:, n * N1:(n + 1) * N1]).astype(BF)

        def mm2(slot, first):
            for n in range(S // N2):
                r = _dot(ubf[...], w2buf[slot, :, n * N2:(n + 1) * N2])
                if first:
                    acc[:, n * N2:(n + 1) * N2] = r
                else:
                    acc[:, n * N2:(n + 1) * N2] += r

        def b1_row(t):
            return b1_ref[pl.ds(pl.multiple_of(t * TF, TF), TF)].astype(F32).reshape(1, TF)

        def conv_fwd(c0):
            for r0 in range(0, CC, PR):
                rows = pl.ds(pl.multiple_of(c0 + r0, 16), PR)
                tp = taps[rows, :]
                w = [jnp.broadcast_to(tp[:, tau:tau + 1], (PR, BL)) for tau in range(KS)]
                ln = lax.broadcasted_iota(jnp.int32, (PR, BL), 1)
                prev = None
                for j in range(J):
                    cols = slice(j * BL, (j + 1) * BL)
                    kb = kT[rows, cols].astype(F32)
                    cur = [pltpu.roll(kb, tau, 1) for tau in range(1, KS)]
                    ksh = kb * w[0]
                    for tau in range(1, KS):
                        fill = jnp.zeros_like(kb) if prev is None else prev[tau - 1]
                        ksh = ksh + jnp.where(ln >= tau, cur[tau - 1], fill) * w[tau]
                    prev = cur
                    kvb[j * CC + r0:j * CC + r0 + PR, :] = (ksh * vT[rows, cols].astype(F32)).astype(BF)
            Xs[...] = _dot(kvb[...], fm_ref[...])
            rows = pl.ds(pl.multiple_of(c0, 16), CC)
            hb = jnp.concatenate([fT[rows, m * BL:(m + 1) * BL] for m in range(J)], axis=0)
            Gs[...] = _dot(hb, fm_ref[...])
            for r0 in range(0, CC, PR):
                dcol = jnp.broadcast_to(taps[pl.ds(pl.multiple_of(c0 + r0, 16), PR), KS:KS + 1], (PR, BL))
                sg = jnp.tile(sgn8, (PR // 8, 1))
                for m in range(J - 1, -1, -1):
                    rm = slice(m * CC + r0, m * CC + r0 + PR)
                    if m == 0:
                        Gs[rm, 0:BL] = Gs[rm, 0:BL] + dcol
                    else:
                        rp = slice((m - 1) * CC + r0, (m - 1) * CC + r0 + PR)
                        Gs[rm, 0:BL] = Gs[rm, 0:BL] - sg * Gs[rp, BL:2 * BL]
                        Gs[rm, BL:2 * BL] = Gs[rm, BL:2 * BL] + sg * Gs[rp, 0:BL]

        def conv_mac():
            for r0 in range(0, CC, MR):
                def ld(ref, j, o):
                    return ref[j * CC + r0:j * CC + r0 + MR, o:o + BL]
                for j in range(J):
                    yr = yi = None
                    for i in range(j + 1):
                        xr, xi = ld(Xs, i, 0), ld(Xs, i, BL)
                        gr, gi = ld(Gs, j - i, 0), ld(Gs, j - i, BL)
                        tr = xr * gr - xi * gi
                        ti = xr * gi + xi * gr
                        yr = tr if yr is None else yr + tr
                        yi = ti if yi is None else yi + ti
                    Ys[j * CC + r0:j * CC + r0 + MR, 0:BL] = yr.astype(BF)
                    Ys[j * CC + r0:j * CC + r0 + MR, BL:2 * BL] = yi.astype(BF)

        def conv_inv(c0):
            rows = pl.ds(pl.multiple_of(c0, 16), CC)
            y = _dot(Ys[...], fi_ref[...])
            for j in range(J):
                cols = slice(j * BL, (j + 1) * BL)
                sT[rows, cols] = (xnT[rows, cols].astype(F32) * y[j * CC:(j + 1) * CC]).astype(BF)

        cp_q(0).wait()
        ln_chunk(0)
        b1r0 = b1_row(0)
        for i in range(NKC):
            if i + 1 < NKC:
                cp_q(i + 1).wait()
            cp_w10(i).wait()
            if i + 1 < NKC:
                ln_chunk(i + 1)
            p = _dot(hT[:, i * KC:(i + 1) * KC], w1buf[0, i * KC:(i + 1) * KC, :])
            if i == 0:
                uacc[...] = p
            elif i + 1 < NKC:
                uacc[...] += p
            else:
                ubf[...] = _gelu(uacc[...] + p + b1r0).astype(BF)
        cp_w2(0, 0).wait()
        mm2(0, True)

        def body(t, _):
            slot = t % 2
            c = t - 1
            cp_w1(t, slot).wait()
            cp_w2(t, slot).wait()
            for cp in cp_kvf(c):
                cp.wait()
            cp_w1(t + 1, 1 - slot).start()
            cp_w2(t + 1, 1 - slot).start()

            @pl.when(t + 1 < NF - 1)
            def _():
                for cp in cp_kvf(c + 1):
                    cp.start()

            c0 = c * CC
            parts = {
                "fwd": lambda: conv_fwd(c0), "mac": conv_mac, "inv": lambda: conv_inv(c0),
                "mm1": lambda: mm1(slot, b1_row(t)), "mm2": lambda: mm2(slot, False),
            }
            for name in order.split(","):
                parts[name]()
            return None

        lax.fori_loop(1, NF - 1, body, None)

        t = NF - 1
        slot = t % 2
        cp_w1(t, slot).wait()
        cp_w2(t, slot).wait()
        mm1(slot, b1_row(t))
        b2row = b2_ref[...].astype(F32).reshape(1, S)
        for n in range(NKC):
            cols = slice(n * KC, (n + 1) * KC)
            y2 = acc[:, cols] + _dot(ubf[...], w2buf[slot, :, cols]) + b2row[:, cols]
            g = (y2 * jax.nn.sigmoid(y2)).astype(BF).astype(F32)
            sg_ = sT[:, cols].astype(F32) * g
            res = sg_ if debug else xT[:, cols].astype(F32) + sg_
            obuf[:, cols] = res.astype(BF)
            cp_o(n).start()
        for n in range(NKC):
            cp_o(n).wait()

    @jax.jit
    def run(A_q, A_k, A_v, A_shift_k, A_ssm_k, A_ssm_D, B_x, B_w1, B_b1, B_w2, B_b2):
        anyspec = pl.BlockSpec(memory_space=pl.ANY)
        vspec = pl.BlockSpec(memory_space=pltpu.VMEM)
        big = pltpu.VMEM((D, S), BF)
        out = pl.pallas_call(
            kernel,
            out_shape=jax.ShapeDtypeStruct((D, S), BF),
            in_specs=[anyspec] * 6 + [vspec] * 6,
            out_specs=anyspec,
            scratch_shapes=[
                big, big, big, big, big, big, big,
                pltpu.VMEM((2, S, TF), BF), pltpu.VMEM((2, TF, S), BF),
                pltpu.VMEM((D, S), F32), pltpu.VMEM((D, TF), F32), pltpu.VMEM((D, TF), BF),
                pltpu.VMEM((J * CC, BL), BF),
                pltpu.VMEM((J * CC, 2 * BL), F32), pltpu.VMEM((J * CC, 2 * BL), F32),
                pltpu.VMEM((J * CC, 2 * BL), BF),
                pltpu.VMEM((640, 128), F32), pltpu.VMEM((128, 640), F32),
                big,
                pltpu.SemaphoreType.DMA((NKC,)), pltpu.SemaphoreType.DMA((NKC,)),
                pltpu.SemaphoreType.DMA((2,)), pltpu.SemaphoreType.DMA((2,)),
                pltpu.SemaphoreType.DMA((3, 2)), pltpu.SemaphoreType.DMA((NKC,)),
            ],
            compiler_params=pltpu.CompilerParams(vmem_limit_bytes=100 * 1024 * 1024),
        )(A_q.reshape(S, D).T, A_k.reshape(S, D).T, A_v.reshape(S, D).T, A_ssm_k, B_w1, B_w2,
          A_shift_k.T, A_ssm_D, B_b1, B_b2, jnp.asarray(FM_NP), jnp.asarray(FI_NP))
        return out.T.reshape(1, S, D)

    return run


_run = build({})


def pallas_recurrent_scan__ssm_conv_h3__mixer_token_mlp__prompt_kernel(
        A_q, A_k, A_v, A_shift_k, A_ssm_k, A_ssm_D, B_x, B_w1, B_b1, B_w2, B_b2):
    return _run(A_q, A_k, A_v, A_shift_k, A_ssm_k, A_ssm_D, B_x, B_w1, B_b1, B_w2, B_b2)
```

```python
import numpy as np
import ml_dtypes
import jax
import jax.numpy as jnp
from jax import lax
import jax.experimental.pallas as pl
import jax.experimental.pallas.tpu as pltpu

S, D, F = 2048, 576, 4608
KS = 4
BL = 128
J = S // BL
KC = 512
NKC = S // KC
EPS = 1e-5
BF = jnp.bfloat16
F32 = jnp.float32

_n = np.arange(BL)[None, :]
_f = np.arange(BL)[:, None]
_th = np.pi * (2 * _f + 1) * _n / (2 * BL)
_FT = np.concatenate([np.cos(_th), -np.sin(_th)], 0)
FM_NP = np.ascontiguousarray(_FT.T).astype(ml_dtypes.bfloat16)
FI_NP = (_FT / BL).astype(ml_dtypes.bfloat16)


def _gelu(x):
    return 0.5 * x * (1.0 + jnp.tanh(0.7978845608028654 * (x + 0.044715 * (x * x * x))))


def _dot(a, b):
    return jnp.dot(a, b, preferred_element_type=F32)


def spread(items, cost, hosts):
    tot = float(sum(cost))
    pos, a = [], 0.0
    for c in cost:
        pos.append(a / tot * len(hosts))
        a += c
    out, k = [], 0
    for hi, h in enumerate(hosts):
        cur = []
        while k < len(items) and pos[k] < hi + 1:
            cur.append((items[k], pos[k] - hi))
            k += 1
        out.append((h, cur))
    return out


def build(cfg):
    TF = cfg.get("TF", 512)
    NF = F // TF
    CC = D // (NF - 1)
    LNC = cfg.get("LNC", 128)
    MR = cfg.get("MR", 8)
    JB = cfg.get("JB", 2)
    PR = cfg.get("PR", 8)
    N1 = cfg.get("N1", 128)
    N2 = cfg.get("N2", 128)
    KQ = cfg.get("KQ", 4)
    GATE = cfg.get("GATE", True)
    GATEP = cfg.get("GATEP", True)
    PFRAC = cfg.get("PFRAC", 0.75)
    MFRAC = cfg.get("MFRAC", 0.95)
    NINV = cfg.get("NINV", 1)
    debug = cfg.get("debug", False)
    import contextlib
    scope = (lambda n: jax.named_scope(n)) if cfg.get("scopes") else (lambda n: contextlib.nullcontext())

    def kernel(q_hbm, k_hbm, v_hbm, f_hbm, w1_hbm, w2_hbm, sk_ref, d_ref, b1_ref, b2_ref, fm_ref, fi_ref,
               o_hbm,
               xT, xnT, hT, kT, vT, fT, sT, w1buf, w2buf, acc, uacc, ubf,
               kvb, Xs, Gs, Ys, taps, tpad, zbuf, obuf,
               sem_q, sem_w10, sem_w1, sem_w2, sem_kvf, sem_o):

        def cp_q(i):
            return pltpu.make_async_copy(q_hbm.at[:, pl.ds(i * KC, KC)], xT.at[:, pl.ds(i * KC, KC)], sem_q.at[i])

        def cp_w10(i):
            return pltpu.make_async_copy(w1_hbm.at[pl.ds(i * KC, KC), pl.ds(0, TF)],
                                         w1buf.at[0, pl.ds(i * KC, KC), :], sem_w10.at[i])

        def cp_w1(t):
            return pltpu.make_async_copy(w1_hbm.at[:, pl.ds(pl.multiple_of(t * TF, TF), TF)], w1buf.at[t % 2], sem_w1.at[t % 2])

        def cp_w2(t):
            return pltpu.make_async_copy(w2_hbm.at[pl.ds(pl.multiple_of(t * TF, TF), TF), :], w2buf.at[t % 2], sem_w2.at[t % 2])

        def cp_kvf(c):
            rows = pl.ds(pl.multiple_of(c * CC, 8), CC)
            return [pltpu.make_async_copy(src.at[rows, :], dst.at[rows, :], sem_kvf.at[a, c % 2])
                    for a, (src, dst) in enumerate(((k_hbm, kT), (v_hbm, vT), (f_hbm, fT)))]

        def cp_o(i):
            return pltpu.make_async_copy(obuf.at[:, pl.ds(i * KC, KC)], o_hbm.at[:, pl.ds(i * KC, KC)], sem_o.at[i])

        for i in range(NKC):
            cp_q(i).start()
            cp_w10(i).start()

        zbuf[...] = jnp.zeros_like(zbuf)
        tpad[...] = jnp.zeros_like(tpad)
        tpad[0:KS, 0:D] = sk_ref[...].astype(F32)
        tpad[KS:KS + 1, 0:D] = d_ref[...].astype(F32).reshape(1, D)
        for ct in range(5):
            taps[ct * 128:(ct + 1) * 128, :] = tpad[:, ct * 128:(ct + 1) * 128].T

        lane = lax.broadcasted_iota(jnp.int32, (8, 128), 1)
        sgn8 = (1 - 2 * (lane & 1)).astype(F32)

        def ln_cols(c0):
            cols = pl.ds(c0, LNC)
            x = xT[:, cols].astype(F32)
            m = jnp.sum(x, axis=0, keepdims=True) * (1.0 / D)
            xc = x - m
            var = jnp.sum(xc * xc, axis=0, keepdims=True) * (1.0 / D)
            xn = (xc * lax.rsqrt(var + EPS)).astype(BF)
            xnT[:, cols] = xn
            xf = xn.astype(F32)
            m2 = jnp.sum(xf, axis=0, keepdims=True) * (1.0 / D)
            xc2 = xf - m2
            var2 = jnp.sum(xc2 * xc2, axis=0, keepdims=True) * (1.0 / D)
            hT[:, cols] = (xc2 * lax.rsqrt(var2 + EPS)).astype(BF)

        def ln_chunk(i):
            for r in range(KC // LNC):
                ln_cols(i * KC + r * LNC)

        def b1_row(t):
            return b1_ref[pl.ds(pl.multiple_of(t * TF, TF), TF)].astype(F32).reshape(1, TF)

        def gate(x, tok):
            if tok is None:
                return x
            t = tok if x.shape[0] == 8 else jnp.tile(tok, (x.shape[0] // 8, 1))
            return pltpu.bitcast(pltpu.bitcast(x, jnp.int32) | t, F32)

        prep_state = {}

        def conv_prep(c0, r0, j0, j1, tok=None):
            rows = pl.ds(pl.multiple_of(c0 + r0, 8), PR)
            tp = taps[rows, :]
            w = [jnp.broadcast_to(tp[:, tau:tau + 1], (PR, BL)) for tau in range(KS)]
            ln = lax.broadcasted_iota(jnp.int32, (PR, BL), 1)
            for j in range(j0, j1):
                cols = slice(j * BL, (j + 1) * BL)
                kb = gate(kT[rows, cols].astype(F32), tok)
                cur = [pltpu.roll(kb, tau, 1) for tau in range(1, KS)]
                ksh = kb * w[0]
                for tau in range(1, KS):
                    sh = cur[tau - 1]
                    if j == 0:
                        sh = jnp.where(ln >= tau, sh, 0.0)
                    else:
                        sh = jnp.where(ln >= tau, sh, prep_state[r0][tau - 1])
                    ksh = ksh + sh * w[tau]
                prep_state[r0] = cur
                kvb[j * CC + r0:j * CC + r0 + PR, :] = (ksh * vT[rows, cols].astype(F32)).astype(BF)

        def conv_dft_x():
            Xs[...] = _dot(kvb[...], fm_ref[...])

        def conv_dft_h(c0):
            rows = pl.ds(pl.multiple_of(c0, 8), CC)
            hb = jnp.concatenate([fT[rows, m * BL:(m + 1) * BL] for m in range(J)], axis=0)
            Gs[...] = _dot(hb, fm_ref[...])

        mac_state = {}

        def conv_mac(c0, r0, jb, tok=None):
            def ld(ref, j, o):
                return ref[j * CC + r0:j * CC + r0 + MR, o:o + BL]
            j0 = jb * JB
            sg = jnp.tile(sgn8, (MR // 8, 1))
            js = list(range(j0, j0 + JB))
            yr = {j: None for j in js}
            yi = {j: None for j in js}
            hwin = {}
            for i in range(js[-1], -1, -1):
                xr, xi = gate(ld(Xs, i, 0), tok), gate(ld(Xs, i, BL), tok)
                for j in js:
                    m = j - i
                    if m < 0:
                        continue
                    if m not in hwin:
                        hr = ld(Gs, m, 0)
                        if m == 0:
                            hr = hr + jnp.broadcast_to(taps[pl.ds(pl.multiple_of(c0 + r0, 8), MR), KS:KS + 1], (MR, BL))
                        hwin[m] = (hr, ld(Gs, m, BL))
                    hr, hi = hwin[m]
                    tr = xr * hr - xi * hi
                    ti = xr * hi + xi * hr
                    yr[j] = tr if yr[j] is None else yr[j] + tr
                    yi[j] = ti if yi[j] is None else yi[j] + ti
            for j in js:
                if j == 0:
                    zr, zi = yr[j], yi[j]
                else:
                    pyr, pyi = mac_state[r0]
                    zr = yr[j] - sg * pyi
                    zi = yi[j] + sg * pyr
                mac_state[r0] = (yr[j], yi[j])
                Ys[j * CC + r0:j * CC + r0 + MR, 0:BL] = zr.astype(Ys.dtype)
                Ys[j * CC + r0:j * CC + r0 + MR, BL:2 * BL] = zi.astype(Ys.dtype)

        def conv_inv(c0, part, nparts):
            rows = pl.ds(pl.multiple_of(c0, 8), CC)
            js = range(part * J // nparts, (part + 1) * J // nparts)
            y = _dot(Ys[js[0] * CC:(js[-1] + 1) * CC, :].astype(BF), fi_ref[...])
            for a_, j in enumerate(js):
                cols = slice(j * BL, (j + 1) * BL)
                sT[rows, cols] = (xnT[rows, cols].astype(F32) * y[a_ * CC:(a_ + 1) * CC]).astype(BF)

        with scope("a_wait_q0"):
            cp_q(0).wait()
        with scope("b_ln0"):
            ln_chunk(0)
        b1r0 = b1_row(0)
        late = [[cp_w1(1)], cp_kvf(0), [cp_w2(0)], []]
        for i in range(NKC):
            with scope("c_wait_s0"):
                if i + 1 < NKC:
                    cp_q(i + 1).wait()
                cp_w10(i).wait()
            for cp in late[i]:
                cp.start()
            with scope("d_s0_mm1"):
                if i + 1 < NKC:
                    ln_chunk(i + 1)
                if i == 1:
                    acc[...] = jnp.zeros_like(acc)
                for n in range(TF // 256):
                    cs = slice(n * 256, (n + 1) * 256)
                    p = _dot(hT[:, i * KC:(i + 1) * KC], w1buf[0, i * KC:(i + 1) * KC, cs])
                    if i == 0:
                        uacc[:, cs] = p
                    elif i + 1 < NKC:
                        uacc[:, cs] += p
                    else:
                        ubf[0, :, cs] = _gelu(uacc[:, cs] + p + b1r0[:, cs]).astype(BF)

        def body(t, _):
            c = t - 1
            c0 = c * CC
            s1 = t % 2
            s2 = (t - 1) % 2
            zmask = zbuf[...]

            def token(v, frac):
                if not GATE:
                    return None
                r8 = min(v.shape[0] // 8 - 1, int(frac * (v.shape[0] // 8)))
                return pltpu.bitcast(v[r8 * 8:r8 * 8 + 8, 0:128], jnp.int32) & zmask

            with scope("g_wait_a"):
                cp_w1(t).wait()
                for cp in cp_kvf(c):
                    cp.wait()

            @pl.when(t + 1 < NF)
            def _():
                cp_w1(t + 1).start()
                for cp in cp_kvf(c + 1):
                    cp.start()

            with scope("h_block_a"):
                b1r = b1_row(t)
                conv_dft_h(c0)
                hosts = [(n, kq) for n in range(TF // N1) for kq in range(KQ)]
                nh = max(1, int(round(len(hosts) * PFRAC)))
                items = [(g, jq) for g in range(CC // PR) for jq in range(4)]
                plan = spread(items, [1] * len(items), hosts[:nh]) + [(h, []) for h in hosts[nh:]]
                u = None
                kw = S // KQ
                for idx, ((n, kq), cur) in enumerate(plan):
                    cs = slice(n * N1, (n + 1) * N1)
                    p = _dot(hT[:, kq * kw:(kq + 1) * kw], w1buf[s1, kq * kw:(kq + 1) * kw, cs])
                    for (g, jq), frac in cur:
                        conv_prep(c0, g * PR, jq * 4, jq * 4 + 4, token(p, frac) if GATEP else None)
                    u = p if kq == 0 else u + p
                    if kq == KQ - 1:
                        ubf[s1, :, cs] = _gelu(u + b1r[:, cs]).astype(BF)
                    if idx == nh - 1:
                        conv_dft_x()

            with scope("i_wait_b"):
                cp_w2(t - 1).wait()
            cp_w2(t).start()

            with scope("j_block_b"):
                hosts = list(range(S // N2))
                nh = max(1, int(round(len(hosts) * MFRAC)))
                items = [(g, jb) for g in range(CC // MR) for jb in range(J // JB)]
                cost = [jb * JB + JB for g, jb in items]
                plan = spread(items, cost, hosts[:nh]) + [(h, []) for h in hosts[nh:]]
                for idx, (n, cur) in enumerate(plan):
                    cs = slice(n * N2, (n + 1) * N2)
                    r = _dot(ubf[s2], w2buf[s2, :, cs])
                    for (g, jb), frac in cur:
                        conv_mac(c0, g * MR, jb, token(r, frac))
                    acc[:, cs] += r
                    if idx == nh - 1:
                        for part in range(NINV):
                            conv_inv(c0, part, NINV)
            return None

        lax.fori_loop(1, NF, body, None)

        t = NF - 1
        with scope("k_wait_last"):
            cp_w2(t).wait()
        b2row = b2_ref[...].astype(F32).reshape(1, S)
        for n in range(NKC):
            with scope("l_epi_%d" % n):
                cols = slice(n * KC, (n + 1) * KC)
                for h in range(KC // 128):
                    cs = slice(n * KC + h * 128, n * KC + (h + 1) * 128)
                    y2 = acc[:, cs] + _dot(ubf[t % 2], w2buf[t % 2, :, cs]) + b2row[:, cs]
                    g = (y2 * jax.nn.sigmoid(y2)).astype(BF).astype(F32)
                    sg_ = sT[:, cs].astype(F32) * g
                    res = sg_ if debug else xT[:, cs].astype(F32) + sg_
                    obuf[:, cs] = res.astype(BF)
                cp_o(n).start()
        with scope("m_out_wait"):
            for n in range(NKC):
                cp_o(n).wait()

    @jax.jit
    def run(A_q, A_k, A_v, A_shift_k, A_ssm_k, A_ssm_D, B_x, B_w1, B_b1, B_w2, B_b2):
        anyspec = pl.BlockSpec(memory_space=pl.ANY)
        vspec = pl.BlockSpec(memory_space=pltpu.VMEM)
        big = pltpu.VMEM((D, S), BF)
        out = pl.pallas_call(
            kernel,
            out_shape=jax.ShapeDtypeStruct((D, S), BF),
            in_specs=[anyspec] * 6 + [vspec] * 6,
            out_specs=anyspec,
            scratch_shapes=[
                big, big, big, big, big, big, big,
                pltpu.VMEM((2, S, TF), BF), pltpu.VMEM((2, TF, S), BF),
                pltpu.VMEM((D, S), F32), pltpu.VMEM((D, TF), F32), pltpu.VMEM((2, D, TF), BF),
                pltpu.VMEM((J * CC, BL), BF),
                pltpu.VMEM((J * CC, 2 * BL), F32), pltpu.VMEM((J * CC, 2 * BL), F32),
                pltpu.VMEM((J * CC, 2 * BL), BF if MR % 16 == 0 else F32),
                pltpu.VMEM((640, 128), F32), pltpu.VMEM((128, 640), F32),
                pltpu.VMEM((8, 128), jnp.int32),
                big,
                pltpu.SemaphoreType.DMA((NKC,)), pltpu.SemaphoreType.DMA((NKC,)),
                pltpu.SemaphoreType.DMA((2,)), pltpu.SemaphoreType.DMA((2,)),
                pltpu.SemaphoreType.DMA((3, 2)), pltpu.SemaphoreType.DMA((NKC,)),
            ],
            compiler_params=pltpu.CompilerParams(vmem_limit_bytes=100 * 1024 * 1024, flags=cfg.get("flags")),
        )(A_q.reshape(S, D).T, A_k.reshape(S, D).T, A_v.reshape(S, D).T, A_ssm_k, B_w1, B_w2,
          A_shift_k.T, A_ssm_D, B_b1, B_b2, jnp.asarray(FM_NP), jnp.asarray(FI_NP))
        return out.T.reshape(1, S, D)

    return run


_run = build({'JB': 4})


def pallas_recurrent_scan__ssm_conv_h3__mixer_token_mlp__prompt_kernel(
        A_q, A_k, A_v, A_shift_k, A_ssm_k, A_ssm_D, B_x, B_w1, B_b1, B_w2, B_b2):
    return _run(A_q, A_k, A_v, A_shift_k, A_ssm_k, A_ssm_D, B_x, B_w1, B_b1, B_w2, B_b2)
```

```python
import numpy as np
import ml_dtypes
import jax
import jax.numpy as jnp
from jax import lax
import jax.experimental.pallas as pl
import jax.experimental.pallas.tpu as pltpu

S, D, F = 2048, 576, 4608
KS = 4
BL = 128
J = S // BL
KC = 512
NKC = S // KC
EPS = 1e-5
BF = jnp.bfloat16
F32 = jnp.float32

_n = np.arange(BL)[None, :]
_f = np.arange(BL)[:, None]
_th = np.pi * (2 * _f + 1) * _n / (2 * BL)
_FT = np.concatenate([np.cos(_th), -np.sin(_th)], 0)
FM_NP = np.ascontiguousarray(_FT.T).astype(ml_dtypes.bfloat16)
FI_NP = (_FT / BL).astype(ml_dtypes.bfloat16)
ZS_NP = np.zeros((8,), np.int32)


def _gelu(x):
    return 0.5 * x * (1.0 + jnp.tanh(0.7978845608028654 * (x + 0.044715 * (x * x * x))))


def _dot(a, b):
    return jnp.dot(a, b, preferred_element_type=F32)


def spread(items, cost, hosts):
    tot = float(sum(cost))
    pos, a = [], 0.0
    for c in cost:
        pos.append(a / tot * len(hosts))
        a += c
    out, k = [], 0
    for hi, h in enumerate(hosts):
        cur = []
        while k < len(items) and pos[k] < hi + 1:
            cur.append((items[k], pos[k] - hi))
            k += 1
        out.append((h, cur))
    return out


def build(cfg):
    TF = cfg.get("TF", 512)
    NF = F // TF
    CC = D // (NF - 1)
    LNC = cfg.get("LNC", 128)
    LNB = cfg.get("LNB", 48)
    GATEL = cfg.get("GATEL", True)
    MERGE = cfg.get("MERGE", False)
    DMAPOS = cfg.get("DMAPOS", -1)
    UNROLL = cfg.get("UNROLL", 1)
    QB = cfg.get("QB", [0, 128, 384, 896, 1408, 2048])
    NQ = len(QB) - 1
    OB = cfg.get("OB", [0, 512, 1024, 1536, 2048])
    NO = len(OB) - 1
    MR = cfg.get("MR", 8)
    JB = cfg.get("JB", 2)
    PR = cfg.get("PR", 8)
    N1 = cfg.get("N1", 128)
    N2 = cfg.get("N2", 128)
    KQ = cfg.get("KQ", 4)
    GATE = cfg.get("GATE", True)
    GATEP = cfg.get("GATEP", True)
    PFRAC = cfg.get("PFRAC", 0.75)
    MFRAC = cfg.get("MFRAC", 0.95)
    NINV = cfg.get("NINV", 1)
    debug = cfg.get("debug", False)
    import contextlib
    scope = (lambda n: jax.named_scope(n)) if cfg.get("scopes") else (lambda n: contextlib.nullcontext())

    def kernel(zs_ref, q_hbm, k_hbm, v_hbm, f_hbm, w1_hbm, w2_hbm, sk_ref, d_ref, b1_ref, b2_ref, fm_ref, fi_ref,
               o_hbm,
               xT, xnT, hT, kT, vT, fT, sT, w1buf, w2buf, acc, uacc, ubf,
               kvb, Xs, Gs, Ys, taps, tpad, zbuf, obuf,
               sem_q, sem_w10, sem_w1, sem_w2, sem_kvf, sem_o):

        def cp_q(i):
            cs = pl.ds(QB[i], QB[i + 1] - QB[i])
            return pltpu.make_async_copy(q_hbm.at[:, cs], xT.at[:, cs], sem_q.at[i])

        def cp_w10(i):
            ks = pl.ds(QB[i], QB[i + 1] - QB[i])
            return pltpu.make_async_copy(w1_hbm.at[ks, pl.ds(0, TF)], w1buf.at[0, ks, :], sem_w10.at[i])

        def cp_w1(t):
            return pltpu.make_async_copy(w1_hbm.at[:, pl.ds(pl.multiple_of(t * TF, TF), TF)], w1buf.at[t % 2], sem_w1.at[t % 2])

        def cp_w2(t):
            return pltpu.make_async_copy(w2_hbm.at[pl.ds(pl.multiple_of(t * TF, TF), TF), :], w2buf.at[t % 2], sem_w2.at[t % 2])

        def cp_kvf(c):
            rows = pl.ds(pl.multiple_of(c * CC, 8), CC)
            return [pltpu.make_async_copy(src.at[rows, :], dst.at[rows, :], sem_kvf.at[a, c % 2])
                    for a, (src, dst) in enumerate(((k_hbm, kT), (v_hbm, vT), (f_hbm, fT)))]

        def cp_o(i):
            cs = pl.ds(OB[i], OB[i + 1] - OB[i])
            return pltpu.make_async_copy(obuf.at[:, cs], o_hbm.at[:, cs], sem_o.at[i])

        for i in range(NQ):
            cp_q(i).start()
            cp_w10(i).start()

        zbuf[...] = jnp.zeros_like(zbuf)
        tpad[...] = jnp.zeros_like(tpad)
        tpad[0:KS, 0:D] = sk_ref[...].astype(F32)
        tpad[KS:KS + 1, 0:D] = d_ref[...].astype(F32).reshape(1, D)
        for ct in range(5):
            taps[ct * 128:(ct + 1) * 128, :] = tpad[:, ct * 128:(ct + 1) * 128].T

        lane = lax.broadcasted_iota(jnp.int32, (8, 128), 1)
        sgn8 = (1 - 2 * (lane & 1)).astype(F32)

        zmask0 = jnp.full((8, 128), zs_ref[3], jnp.int32)

        def gate16(x, tok):
            if tok is None:
                return x
            xi = pltpu.bitcast(x, jnp.int32)
            return pltpu.bitcast(xi | jnp.tile(tok, (xi.shape[0] // 8, 1)), BF)

        def ln_steps(lo, hi):
            for c0 in range(lo, hi, 128):
                cols = pl.ds(c0, 128)
                starts = range(0, D, LNB)

                def ldx(r, k, tok):
                    rows = pl.ds(r, LNB) if k is None else pl.ds(pl.multiple_of(r + zs_ref[k], 16), LNB)
                    return gate16(xT[rows, cols], tok).astype(F32)

                def fold(t, v):
                    for g in range(LNB // 8):
                        p_ = v[g * 8:(g + 1) * 8]
                        t = p_ if t is None else t + p_
                    return t

                t = None
                for r in starts:
                    tok = yield
                    t = fold(t, ldx(r, None, tok))
                m = jnp.sum(t, axis=0, keepdims=True) * (1.0 / D)
                t = None
                for r in starts:
                    tok = yield
                    xc = ldx(r, 0, tok) - m
                    t = fold(t, xc * xc)
                var = jnp.sum(t, axis=0, keepdims=True) * (1.0 / D)
                rs = lax.rsqrt(var + EPS)
                rsh = rs * lax.rsqrt(var * rs * rs + EPS)
                for r in starts:
                    tok = yield
                    xc = ldx(r, 1, tok) - m
                    xnT[pl.ds(r, LNB), cols] = (xc * rs).astype(BF)
                    hT[pl.ds(r, LNB), cols] = (xc * rsh).astype(BF)

        def ln_nsteps(lo, hi):
            return (hi - lo) // 128 * 3 * (D // LNB)

        def ln_run(lo, hi):
            gen = ln_steps(lo, hi)
            next(gen)
            for _ in range(ln_nsteps(lo, hi) - 1):
                gen.send(None)
            try:
                gen.send(None)
            except StopIteration:
                pass

        def b1_row(t):
            return b1_ref[pl.ds(pl.multiple_of(t * TF, TF), TF)].astype(F32).reshape(1, TF)

        def gate(x, tok):
            if tok is None:
                return x
            t = tok if x.shape[0] == 8 else jnp.tile(tok, (x.shape[0] // 8, 1))
            return pltpu.bitcast(pltpu.bitcast(x, jnp.int32) | t, F32)

        prep_state = {}

        def conv_prep(c0, r0, j0, j1, tok=None):
            rows = pl.ds(pl.multiple_of(c0 + r0, 8), PR)
            tp = taps[rows, :]
            w = [jnp.broadcast_to(tp[:, tau:tau + 1], (PR, BL)) for tau in range(KS)]
            ln = lax.broadcasted_iota(jnp.int32, (PR, BL), 1)
            for j in range(j0, j1):
                cols = slice(j * BL, (j + 1) * BL)
                kb = gate(kT[rows, cols].astype(F32), tok)
                cur = [pltpu.roll(kb, tau, 1) for tau in range(1, KS)]
                ksh = kb * w[0]
                for tau in range(1, KS):
                    sh = cur[tau - 1]
                    if j == 0:
                        sh = jnp.where(ln >= tau, sh, 0.0)
                    else:
                        sh = jnp.where(ln >= tau, sh, prep_state[r0][tau - 1])
                    ksh = ksh + sh * w[tau]
                prep_state[r0] = cur
                kvb[j * CC + r0:j * CC + r0 + PR, :] = (ksh * vT[rows, cols].astype(F32)).astype(BF)

        def conv_dft_x():
            Xs[...] = _dot(kvb[...], fm_ref[...])

        def conv_dft_h(c0):
            rows = pl.ds(pl.multiple_of(c0, 8), CC)
            hb = jnp.concatenate([fT[rows, m * BL:(m + 1) * BL] for m in range(J)], axis=0)
            Gs[...] = _dot(hb, fm_ref[...])

        mac_state = {}

        def conv_mac(c0, r0, jb, tok=None):
            def ld(ref, j, o):
                return ref[j * CC + r0:j * CC + r0 + MR, o:o + BL]
            j0 = jb * JB
            sg = jnp.tile(sgn8, (MR // 8, 1))
            js = list(range(j0, j0 + JB))
            yr = {j: None for j in js}
            yi = {j: None for j in js}
            hwin = {}
            for i in range(js[-1], -1, -1):
                xr, xi = gate(ld(Xs, i, 0), tok), gate(ld(Xs, i, BL), tok)
                for j in js:
                    m = j - i
                    if m < 0:
                        continue
                    if m not in hwin:
                        hr = ld(Gs, m, 0)
                        if m == 0:
                            hr = hr + jnp.broadcast_to(taps[pl.ds(pl.multiple_of(c0 + r0, 8), MR), KS:KS + 1], (MR, BL))
                        hwin[m] = (hr, ld(Gs, m, BL))
                    hr, hi = hwin[m]
                    tr = xr * hr - xi * hi
                    ti = xr * hi + xi * hr
                    yr[j] = tr if yr[j] is None else yr[j] + tr
                    yi[j] = ti if yi[j] is None else yi[j] + ti
            for j in js:
                if j == 0:
                    zr, zi = yr[j], yi[j]
                else:
                    pyr, pyi = mac_state[r0]
                    zr = yr[j] - sg * pyi
                    zi = yi[j] + sg * pyr
                mac_state[r0] = (yr[j], yi[j])
                Ys[j * CC + r0:j * CC + r0 + MR, 0:BL] = zr.astype(Ys.dtype)
                Ys[j * CC + r0:j * CC + r0 + MR, BL:2 * BL] = zi.astype(Ys.dtype)

        def conv_inv(c0, part, nparts):
            rows = pl.ds(pl.multiple_of(c0, 8), CC)
            js = range(part * J // nparts, (part + 1) * J // nparts)
            y = _dot(Ys[js[0] * CC:(js[-1] + 1) * CC, :].astype(BF), fi_ref[...])
            for a_, j in enumerate(js):
                cols = slice(j * BL, (j + 1) * BL)
                sT[rows, cols] = (xnT[rows, cols].astype(F32) * y[a_ * CC:(a_ + 1) * CC]).astype(BF)

        with scope("a_wait_q0"):
            cp_q(0).wait()
        with scope("b_ln0"):
            ln_run(QB[0], QB[1])
        b1r0 = b1_row(0)
        late = {1: [cp_w1(1)], 2: cp_kvf(0), 3: [cp_w2(0)]}
        for i in range(NQ):
            with scope("c_wait_s0"):
                if i + 1 < NQ:
                    cp_q(i + 1).wait()
                cp_w10(i).wait()
            for cp in late.get(i, []):
                cp.start()
            with scope("d_s0_mm1"):
                ks = slice(QB[i], QB[i + 1])
                hosts = list(range(TF // 128))
                if i + 1 < NQ:
                    gen = ln_steps(QB[i + 1], QB[i + 2])
                    next(gen)
                    ns = ln_nsteps(QB[i + 1], QB[i + 2])
                    plan = spread(list(range(ns)), [1] * ns, hosts)
                else:
                    gen = None
                    plan = [(h, []) for h in hosts]
                for n, cur in plan:
                    cs = slice(n * 128, (n + 1) * 128)
                    p = _dot(hT[:, ks], w1buf[0, ks, cs])
                    for _, frac in cur:
                        tok = None
                        if GATEL:
                            r8 = min(71, int(frac * 72))
                            tok = pltpu.bitcast(p[r8 * 8:r8 * 8 + 8, :], jnp.int32) & zmask0
                        try:
                            gen.send(tok)
                        except StopIteration:
                            pass
                    if i == 0:
                        uacc[:, cs] = p
                    elif i + 1 < NQ:
                        uacc[:, cs] += p
                    else:
                        ubf[0, :, cs] = _gelu(uacc[:, cs] + p + b1r0[:, cs]).astype(BF)
                if i == NQ - 1:
                    acc[...] = jnp.zeros_like(acc)

        def body(t, _):
            c = t - 1
            c0 = c * CC
            s1 = t % 2
            s2 = (t - 1) % 2
            zmask = zmask0

            def token(v, frac):
                if not GATE:
                    return None
                r8 = min(v.shape[0] // 8 - 1, int(frac * (v.shape[0] // 8)))
                return pltpu.bitcast(v[r8 * 8:r8 * 8 + 8, 0:128], jnp.int32) & zmask

            with scope("g_wait_a"):
                cp_w1(t).wait()
                for cp in cp_kvf(c):
                    cp.wait()
                if MERGE:
                    cp_w2(t - 1).wait()
            if MERGE:
                cp_w2(t).start()

            def prefetch_a():
                @pl.when(t + 1 < NF)
                def _():
                    cp_w1(t + 1).start()
                    for cp in cp_kvf(c + 1):
                        cp.start()

            if DMAPOS < 0:
                prefetch_a()

            with scope("h_block_a"):
                b1r = b1_row(t)
                conv_dft_h(c0)
                hosts = [(n, kq) for n in range(TF // N1) for kq in range(KQ)]
                nh = max(1, int(round(len(hosts) * PFRAC)))
                items = [(g, jq) for g in range(CC // PR) for jq in range(4)]
                plan = spread(items, [1] * len(items), hosts[:nh]) + [(h, []) for h in hosts[nh:]]
                u = None
                kw = S // KQ
                for idx, ((n, kq), cur) in enumerate(plan):
                    cs = slice(n * N1, (n + 1) * N1)
                    p = _dot(hT[:, kq * kw:(kq + 1) * kw], w1buf[s1, kq * kw:(kq + 1) * kw, cs])
                    for (g, jq), frac in cur:
                        conv_prep(c0, g * PR, jq * 4, jq * 4 + 4, token(p, frac) if GATEP else None)
                    u = p if kq == 0 else u + p
                    if kq == KQ - 1:
                        ubf[s1, :, cs] = _gelu(u + b1r[:, cs]).astype(BF)
                    if idx == nh - 1:
                        conv_dft_x()
                    if idx == DMAPOS:
                        prefetch_a()

            if not MERGE:
                with scope("i_wait_b"):
                    cp_w2(t - 1).wait()
                if DMAPOS < 0:
                    cp_w2(t).start()

            with scope("j_block_b"):
                hosts = list(range(S // N2))
                nh = max(1, int(round(len(hosts) * MFRAC)))
                items = [(g, jb) for g in range(CC // MR) for jb in range(J // JB)]
                cost = [jb * JB + JB for g, jb in items]
                plan = spread(items, cost, hosts[:nh]) + [(h, []) for h in hosts[nh:]]
                for idx, (n, cur) in enumerate(plan):
                    cs = slice(n * N2, (n + 1) * N2)
                    r = _dot(ubf[s2], w2buf[s2, :, cs])
                    for (g, jb), frac in cur:
                        conv_mac(c0, g * MR, jb, token(r, frac))
                    acc[:, cs] += r
                    if (not MERGE) and idx == DMAPOS:
                        cp_w2(t).start()
                    if idx == nh - 1:
                        for part in range(NINV):
                            conv_inv(c0, part, NINV)
            return None

        lax.fori_loop(1, NF, body, None, unroll=UNROLL)

        t = NF - 1
        with scope("k_wait_last"):
            cp_w2(t).wait()
        b2row = b2_ref[...].astype(F32).reshape(1, S)
        for n in range(NO):
            with scope("l_epi_%d" % n):
                for c_ in range(OB[n], OB[n + 1], 128):
                    cs = slice(c_, c_ + 128)
                    y2 = acc[:, cs] + _dot(ubf[t % 2], w2buf[t % 2, :, cs]) + b2row[:, cs]
                    g = (y2 * jax.nn.sigmoid(y2)).astype(BF).astype(F32)
                    sg_ = sT[:, cs].astype(F32) * g
                    res = sg_ if debug else xT[:, cs].astype(F32) + sg_
                    obuf[:, cs] = res.astype(BF)
                cp_o(n).start()
        with scope("m_out_wait"):
            for n in range(NO):
                cp_o(n).wait()

    @jax.jit
    def run(A_q, A_k, A_v, A_shift_k, A_ssm_k, A_ssm_D, B_x, B_w1, B_b1, B_w2, B_b2):
        anyspec = pl.BlockSpec(memory_space=pl.ANY)
        vspec = pl.BlockSpec(memory_space=pltpu.VMEM)
        big = pltpu.VMEM((D, S), BF)
        out = pl.pallas_call(
            kernel,
            out_shape=jax.ShapeDtypeStruct((D, S), BF),
            in_specs=[pl.BlockSpec(memory_space=pltpu.SMEM)] + [anyspec] * 6 + [vspec] * 6,
            out_specs=anyspec,
            scratch_shapes=[
                big, big, big, big, big, big, big,
                pltpu.VMEM((2, S, TF), BF), pltpu.VMEM((2, TF, S), BF),
                pltpu.VMEM((D, S), F32), pltpu.VMEM((D, TF), F32), pltpu.VMEM((2, D, TF), BF),
                pltpu.VMEM((J * CC, BL), BF),
                pltpu.VMEM((J * CC, 2 * BL), F32), pltpu.VMEM((J * CC, 2 * BL), F32),
                pltpu.VMEM((J * CC, 2 * BL), BF if MR % 16 == 0 else F32),
                pltpu.VMEM((640, 128), F32), pltpu.VMEM((128, 640), F32),
                pltpu.VMEM((8, 128), jnp.int32),
                big,
                pltpu.SemaphoreType.DMA((NQ,)), pltpu.SemaphoreType.DMA((NQ,)),
                pltpu.SemaphoreType.DMA((2,)), pltpu.SemaphoreType.DMA((2,)),
                pltpu.SemaphoreType.DMA((3, 2)), pltpu.SemaphoreType.DMA((NO,)),
            ],
            compiler_params=pltpu.CompilerParams(vmem_limit_bytes=100 * 1024 * 1024, flags=cfg.get("flags")),
        )(jnp.asarray(ZS_NP), A_q.reshape(S, D).T, A_k.reshape(S, D).T, A_v.reshape(S, D).T, A_ssm_k, B_w1, B_w2,
          A_shift_k.T, A_ssm_D, B_b1, B_b2, jnp.asarray(FM_NP), jnp.asarray(FI_NP))
        return out.T.reshape(1, S, D)

    return run


_run = build({'JB': 4, 'OB': [0, 512, 1024, 1536, 1792, 1920, 2048], 'DMAPOS': 1})


def pallas_recurrent_scan__ssm_conv_h3__mixer_token_mlp__prompt_kernel(
        A_q, A_k, A_v, A_shift_k, A_ssm_k, A_ssm_D, B_x, B_w1, B_b1, B_w2, B_b2):
    return _run(A_q, A_k, A_v, A_shift_k, A_ssm_k, A_ssm_D, B_x, B_w1, B_b1, B_w2, B_b2)
```

```python
import numpy as np
import ml_dtypes
import jax
import jax.numpy as jnp
from jax import lax
import jax.experimental.pallas as pl
import jax.experimental.pallas.tpu as pltpu

S, D, F = 2048, 576, 4608
KS = 4
BL = 128
J = S // BL
EPS = 1e-5
BF = jnp.bfloat16
F32 = jnp.float32

_n = np.arange(BL)[None, :]
_f = np.arange(BL)[:, None]
_th = np.pi * (2 * _f + 1) * _n / (2 * BL)
_FT = np.concatenate([np.cos(_th), -np.sin(_th)], 0)
FM_NP = np.ascontiguousarray(_FT.T).astype(ml_dtypes.bfloat16)
FI_NP = (_FT / BL).astype(ml_dtypes.bfloat16)
ZS_NP = np.zeros((8,), np.int32)


def _gelu(x):
    return 0.5 * x * (1.0 + jnp.tanh(0.7978845608028654 * (x + 0.044715 * (x * x * x))))


def _dot(a, b):
    return jnp.dot(a, b, preferred_element_type=F32)


def spread(items, cost, hosts):
    tot = float(sum(cost))
    pos, a = [], 0.0
    for c in cost:
        pos.append(a / tot * len(hosts))
        a += c
    out, k = [], 0
    for hi, h in enumerate(hosts):
        cur = []
        while k < len(items) and pos[k] < hi + 1:
            cur.append((items[k], pos[k] - hi))
            k += 1
        out.append((h, cur))
    return out


TF = 512
NF = F // TF
CC = D // (NF - 1)
LNB = 48
QB = (0, 128, 384, 896, 1408, 2048)
NQ = len(QB) - 1
OB = (0, 512, 1024, 1536, 1792, 1920, 2048)
NO = len(OB) - 1
MR = 8
JB = 4
PR = 8
N1 = 128
N2 = 128
KQ = 4
PFRAC = 0.75
MFRAC = 0.95
DMAPOS = 1


def _build():
    def kernel(zs_ref, q_hbm, k_hbm, v_hbm, f_hbm, w1_hbm, w2_hbm, sk_ref, d_ref, b1_ref, b2_ref, fm_ref, fi_ref,
               o_hbm,
               xT, xnT, hT, kT, vT, fT, sT, w1buf, w2buf, acc, uacc, ubf,
               kvb, Xs, Gs, Ys, taps, tpad, obuf,
               sem_q, sem_w10, sem_w1, sem_w2, sem_kvf, sem_o):

        def cp_q(i):
            cs = pl.ds(QB[i], QB[i + 1] - QB[i])
            return pltpu.make_async_copy(q_hbm.at[:, cs], xT.at[:, cs], sem_q.at[i])

        def cp_w10(i):
            ks = pl.ds(QB[i], QB[i + 1] - QB[i])
            return pltpu.make_async_copy(w1_hbm.at[ks, pl.ds(0, TF)], w1buf.at[0, ks, :], sem_w10.at[i])

        def cp_w1(t):
            return pltpu.make_async_copy(w1_hbm.at[:, pl.ds(pl.multiple_of(t * TF, TF), TF)], w1buf.at[t % 2], sem_w1.at[t % 2])

        def cp_w2(t):
            return pltpu.make_async_copy(w2_hbm.at[pl.ds(pl.multiple_of(t * TF, TF), TF), :], w2buf.at[t % 2], sem_w2.at[t % 2])

        def cp_kvf(c):
            rows = pl.ds(pl.multiple_of(c * CC, 8), CC)
            return [pltpu.make_async_copy(src.at[rows, :], dst.at[rows, :], sem_kvf.at[a, c % 2])
                    for a, (src, dst) in enumerate(((k_hbm, kT), (v_hbm, vT), (f_hbm, fT)))]

        def cp_o(i):
            cs = pl.ds(OB[i], OB[i + 1] - OB[i])
            return pltpu.make_async_copy(obuf.at[:, cs], o_hbm.at[:, cs], sem_o.at[i])

        for i in range(NQ):
            cp_q(i).start()
            cp_w10(i).start()

        tpad[...] = jnp.zeros_like(tpad)
        tpad[0:KS, 0:D] = sk_ref[...].astype(F32)
        tpad[KS:KS + 1, 0:D] = d_ref[...].astype(F32).reshape(1, D)
        for ct in range(5):
            taps[ct * 128:(ct + 1) * 128, :] = tpad[:, ct * 128:(ct + 1) * 128].T

        lane = lax.broadcasted_iota(jnp.int32, (8, 128), 1)
        sgn8 = (1 - 2 * (lane & 1)).astype(F32)

        zmask0 = jnp.full((8, 128), zs_ref[3], jnp.int32)

        def token(v, frac):
            r8 = min(v.shape[0] // 8 - 1, int(frac * (v.shape[0] // 8)))
            return pltpu.bitcast(v[r8 * 8:r8 * 8 + 8, 0:128], jnp.int32) & zmask0

        def gate16(x, tok):
            if tok is None:
                return x
            xi = pltpu.bitcast(x, jnp.int32)
            return pltpu.bitcast(xi | jnp.tile(tok, (xi.shape[0] // 8, 1)), BF)

        def ln_steps(lo, hi):
            for c0 in range(lo, hi, 128):
                cols = pl.ds(c0, 128)
                starts = range(0, D, LNB)

                def ldx(r, k, tok):
                    rows = pl.ds(r, LNB) if k is None else pl.ds(pl.multiple_of(r + zs_ref[k], 16), LNB)
                    return gate16(xT[rows, cols], tok).astype(F32)

                def fold(t, v):
                    for g in range(LNB // 8):
                        p_ = v[g * 8:(g + 1) * 8]
                        t = p_ if t is None else t + p_
                    return t

                t = None
                for r in starts:
                    tok = yield
                    t = fold(t, ldx(r, None, tok))
                m = jnp.sum(t, axis=0, keepdims=True) * (1.0 / D)
                t = None
                for r in starts:
                    tok = yield
                    xc = ldx(r, 0, tok) - m
                    t = fold(t, xc * xc)
                var = jnp.sum(t, axis=0, keepdims=True) * (1.0 / D)
                rs = lax.rsqrt(var + EPS)
                rsh = rs * lax.rsqrt(var * rs * rs + EPS)
                for r in starts:
                    tok = yield
                    xc = ldx(r, 1, tok) - m
                    xnT[pl.ds(r, LNB), cols] = (xc * rs).astype(BF)
                    hT[pl.ds(r, LNB), cols] = (xc * rsh).astype(BF)

        def ln_nsteps(lo, hi):
            return (hi - lo) // 128 * 3 * (D // LNB)

        def ln_run(lo, hi):
            gen = ln_steps(lo, hi)
            next(gen)
            for _ in range(ln_nsteps(lo, hi) - 1):
                gen.send(None)
            try:
                gen.send(None)
            except StopIteration:
                pass

        def b1_row(t):
            return b1_ref[pl.ds(pl.multiple_of(t * TF, TF), TF)].astype(F32).reshape(1, TF)

        def gate(x, tok):
            if tok is None:
                return x
            t = tok if x.shape[0] == 8 else jnp.tile(tok, (x.shape[0] // 8, 1))
            return pltpu.bitcast(pltpu.bitcast(x, jnp.int32) | t, F32)

        prep_state = {}

        def conv_prep(c0, r0, j0, j1, tok=None):
            rows = pl.ds(pl.multiple_of(c0 + r0, 8), PR)
            tp = taps[rows, :]
            w = [jnp.broadcast_to(tp[:, tau:tau + 1], (PR, BL)) for tau in range(KS)]
            ln = lax.broadcasted_iota(jnp.int32, (PR, BL), 1)
            for j in range(j0, j1):
                cols = slice(j * BL, (j + 1) * BL)
                kb = gate(kT[rows, cols].astype(F32), tok)
                cur = [pltpu.roll(kb, tau, 1) for tau in range(1, KS)]
                ksh = kb * w[0]
                for tau in range(1, KS):
                    sh = cur[tau - 1]
                    if j == 0:
                        sh = jnp.where(ln >= tau, sh, 0.0)
                    else:
                        sh = jnp.where(ln >= tau, sh, prep_state[r0][tau - 1])
                    ksh = ksh + sh * w[tau]
                prep_state[r0] = cur
                kvb[j * CC + r0:j * CC + r0 + PR, :] = (ksh * vT[rows, cols].astype(F32)).astype(BF)

        def conv_dft_x():
            Xs[...] = _dot(kvb[...], fm_ref[...])

        def conv_dft_h(c0):
            rows = pl.ds(pl.multiple_of(c0, 8), CC)
            hb = jnp.concatenate([fT[rows, m * BL:(m + 1) * BL] for m in range(J)], axis=0)
            Gs[...] = _dot(hb, fm_ref[...])

        mac_state = {}

        def conv_mac(c0, r0, jb, tok=None):
            def ld(ref, j, o):
                return ref[j * CC + r0:j * CC + r0 + MR, o:o + BL]
            j0 = jb * JB
            sg = jnp.tile(sgn8, (MR // 8, 1))
            js = list(range(j0, j0 + JB))
            yr = {j: None for j in js}
            yi = {j: None for j in js}
            hwin = {}
            for i in range(js[-1], -1, -1):
                xr, xi = gate(ld(Xs, i, 0), tok), gate(ld(Xs, i, BL), tok)
                for j in js:
                    m = j - i
                    if m < 0:
                        continue
                    if m not in hwin:
                        hr = ld(Gs, m, 0)
                        if m == 0:
                            hr = hr + jnp.broadcast_to(taps[pl.ds(pl.multiple_of(c0 + r0, 8), MR), KS:KS + 1], (MR, BL))
                        hwin[m] = (hr, ld(Gs, m, BL))
                    hr, hi = hwin[m]
                    tr = xr * hr - xi * hi
                    ti = xr * hi + xi * hr
                    yr[j] = tr if yr[j] is None else yr[j] + tr
                    yi[j] = ti if yi[j] is None else yi[j] + ti
            for j in js:
                if j == 0:
                    zr, zi = yr[j], yi[j]
                else:
                    pyr, pyi = mac_state[r0]
                    zr = yr[j] - sg * pyi
                    zi = yi[j] + sg * pyr
                mac_state[r0] = (yr[j], yi[j])
                Ys[j * CC + r0:j * CC + r0 + MR, 0:BL] = zr.astype(Ys.dtype)
                Ys[j * CC + r0:j * CC + r0 + MR, BL:2 * BL] = zi.astype(Ys.dtype)

        def conv_inv(c0):
            rows = pl.ds(pl.multiple_of(c0, 8), CC)
            y = _dot(Ys[...].astype(BF), fi_ref[...])
            for j in range(J):
                cols = slice(j * BL, (j + 1) * BL)
                sT[rows, cols] = (xnT[rows, cols].astype(F32) * y[j * CC:(j + 1) * CC]).astype(BF)

        cp_q(0).wait()
        ln_run(QB[0], QB[1])
        b1r0 = b1_row(0)
        late = {1: [cp_w1(1)], 2: cp_kvf(0), 3: [cp_w2(0)]}
        for i in range(NQ):
            if i + 1 < NQ:
                cp_q(i + 1).wait()
            cp_w10(i).wait()
            for cp in late.get(i, []):
                cp.start()
            ks = slice(QB[i], QB[i + 1])
            hosts = list(range(TF // 128))
            if i + 1 < NQ:
                gen = ln_steps(QB[i + 1], QB[i + 2])
                next(gen)
                ns = ln_nsteps(QB[i + 1], QB[i + 2])
                plan = spread(list(range(ns)), [1] * ns, hosts)
            else:
                gen = None
                plan = [(h, []) for h in hosts]
            for n, cur in plan:
                cs = slice(n * 128, (n + 1) * 128)
                p = _dot(hT[:, ks], w1buf[0, ks, cs])
                for _, frac in cur:
                    try:
                        gen.send(token(p, frac))
                    except StopIteration:
                        pass
                if i == 0:
                    uacc[:, cs] = p
                elif i + 1 < NQ:
                    uacc[:, cs] += p
                else:
                    ubf[0, :, cs] = _gelu(uacc[:, cs] + p + b1r0[:, cs]).astype(BF)
            if i == NQ - 1:
                acc[...] = jnp.zeros_like(acc)

        def body(t, _):
            c = t - 1
            c0 = c * CC
            s1 = t % 2
            s2 = (t - 1) % 2

            cp_w1(t).wait()
            for cp in cp_kvf(c):
                cp.wait()

            def prefetch_a():
                @pl.when(t + 1 < NF)
                def _():
                    cp_w1(t + 1).start()
                    for cp in cp_kvf(c + 1):
                        cp.start()

            b1r = b1_row(t)
            conv_dft_h(c0)
            hosts = [(n, kq) for n in range(TF // N1) for kq in range(KQ)]
            nh = max(1, int(round(len(hosts) * PFRAC)))
            items = [(g, jq) for g in range(CC // PR) for jq in range(4)]
            plan = spread(items, [1] * len(items), hosts[:nh]) + [(h, []) for h in hosts[nh:]]
            u = None
            kw = S // KQ
            for idx, ((n, kq), cur) in enumerate(plan):
                cs = slice(n * N1, (n + 1) * N1)
                p = _dot(hT[:, kq * kw:(kq + 1) * kw], w1buf[s1, kq * kw:(kq + 1) * kw, cs])
                for (g, jq), frac in cur:
                    conv_prep(c0, g * PR, jq * 4, jq * 4 + 4, token(p, frac))
                u = p if kq == 0 else u + p
                if kq == KQ - 1:
                    ubf[s1, :, cs] = _gelu(u + b1r[:, cs]).astype(BF)
                if idx == nh - 1:
                    conv_dft_x()
                if idx == DMAPOS:
                    prefetch_a()

            cp_w2(t - 1).wait()

            hosts = list(range(S // N2))
            nh = max(1, int(round(len(hosts) * MFRAC)))
            items = [(g, jb) for g in range(CC // MR) for jb in range(J // JB)]
            cost = [jb * JB + JB for g, jb in items]
            plan = spread(items, cost, hosts[:nh]) + [(h, []) for h in hosts[nh:]]
            for idx, (n, cur) in enumerate(plan):
                cs = slice(n * N2, (n + 1) * N2)
                r = _dot(ubf[s2], w2buf[s2, :, cs])
                for (g, jb), frac in cur:
                    conv_mac(c0, g * MR, jb, token(r, frac))
                acc[:, cs] += r
                if idx == DMAPOS:
                    cp_w2(t).start()
                if idx == nh - 1:
                    conv_inv(c0)
            return None

        lax.fori_loop(1, NF, body, None)

        t = NF - 1
        cp_w2(t).wait()
        b2row = b2_ref[...].astype(F32).reshape(1, S)
        for n in range(NO):
            for c_ in range(OB[n], OB[n + 1], 128):
                cs = slice(c_, c_ + 128)
                y2 = acc[:, cs] + _dot(ubf[t % 2], w2buf[t % 2, :, cs]) + b2row[:, cs]
                g = (y2 * jax.nn.sigmoid(y2)).astype(BF).astype(F32)
                sg_ = sT[:, cs].astype(F32) * g
                obuf[:, cs] = (xT[:, cs].astype(F32) + sg_).astype(BF)
            cp_o(n).start()
        for n in range(NO):
            cp_o(n).wait()

    def run(A_q, A_k, A_v, A_shift_k, A_ssm_k, A_ssm_D, B_x, B_w1, B_b1, B_w2, B_b2):
        anyspec = pl.BlockSpec(memory_space=pl.ANY)
        vspec = pl.BlockSpec(memory_space=pltpu.VMEM)
        big = pltpu.VMEM((D, S), BF)
        out = pl.pallas_call(
            kernel,
            out_shape=jax.ShapeDtypeStruct((D, S), BF),
            in_specs=[pl.BlockSpec(memory_space=pltpu.SMEM)] + [anyspec] * 6 + [vspec] * 6,
            out_specs=anyspec,
            scratch_shapes=[
                big, big, big, big, big, big, big,
                pltpu.VMEM((2, S, TF), BF), pltpu.VMEM((2, TF, S), BF),
                pltpu.VMEM((D, S), F32), pltpu.VMEM((D, TF), F32), pltpu.VMEM((2, D, TF), BF),
                pltpu.VMEM((J * CC, BL), BF),
                pltpu.VMEM((J * CC, 2 * BL), F32), pltpu.VMEM((J * CC, 2 * BL), F32),
                pltpu.VMEM((J * CC, 2 * BL), F32),
                pltpu.VMEM((640, 128), F32), pltpu.VMEM((128, 640), F32),
                big,
                pltpu.SemaphoreType.DMA((NQ,)), pltpu.SemaphoreType.DMA((NQ,)),
                pltpu.SemaphoreType.DMA((2,)), pltpu.SemaphoreType.DMA((2,)),
                pltpu.SemaphoreType.DMA((3, 2)), pltpu.SemaphoreType.DMA((NO,)),
            ],
            compiler_params=pltpu.CompilerParams(vmem_limit_bytes=100 * 1024 * 1024),
        )(jnp.asarray(ZS_NP), A_q.reshape(S, D).T, A_k.reshape(S, D).T, A_v.reshape(S, D).T, A_ssm_k, B_w1, B_w2,
          A_shift_k.T, A_ssm_D, B_b1, B_b2, jnp.asarray(FM_NP), jnp.asarray(FI_NP))
        return out.T.reshape(1, S, D)

    return run


_run = _build()


@jax.jit
def pallas_recurrent_scan__ssm_conv_h3__mixer_token_mlp__prompt_kernel(
        A_q, A_k, A_v, A_shift_k, A_ssm_k, A_ssm_D, B_x, B_w1, B_b1, B_w2, B_b2):
    return _run(A_q, A_k, A_v, A_shift_k, A_ssm_k, A_ssm_D, B_x, B_w1, B_b1, B_w2, B_b2)
```

```python
import numpy as np
import ml_dtypes
import jax
import jax.numpy as jnp
from jax import lax
import jax.experimental.pallas as pl
import jax.experimental.pallas.tpu as pltpu

S, D, F = 2048, 576, 4608
KS = 4
BL = 128
J = S // BL
EPS = 1e-5
BF = jnp.bfloat16
F32 = jnp.float32

_n = np.arange(BL)[None, :]
_f = np.arange(BL)[:, None]
_th = np.pi * (2 * _f + 1) * _n / (2 * BL)
_FT = np.concatenate([np.cos(_th), -np.sin(_th)], 0)
FM_NP = np.ascontiguousarray(_FT.T).astype(ml_dtypes.bfloat16)
FI_NP = (_FT / BL).astype(ml_dtypes.bfloat16)
ZS_NP = np.zeros((8,), np.int32)


def _gelu(x):
    return 0.5 * x * (1.0 + jnp.tanh(0.7978845608028654 * (x + 0.044715 * (x * x * x))))


def _dot(a, b):
    return jnp.dot(a, b, preferred_element_type=F32)


def spread(items, cost, hosts):
    tot = float(sum(cost))
    pos, a = [], 0.0
    for c in cost:
        pos.append(a / tot * len(hosts))
        a += c
    out, k = [], 0
    for hi, h in enumerate(hosts):
        cur = []
        while k < len(items) and pos[k] < hi + 1:
            cur.append((items[k], pos[k] - hi))
            k += 1
        out.append((h, cur))
    return out


TF = 512
NF = F // TF
CC = D // (NF - 1)
LNB = 48
QB = (0, 128, 384, 896, 1408, 2048)
NQ = len(QB) - 1
OB = (0, 512, 1024, 1536, 1792, 1920, 2048)
NO = len(OB) - 1
MR = 8
JB = 4
PJ = 2
N1 = 128
N2 = 128
KQ = 4
PFRAC = 0.75
MFRAC = 0.95
DMAPOS = 1


def _build():
    def kernel(zs_ref, q_hbm, k_hbm, v_hbm, f_hbm, w1_hbm, w2_hbm, sk_ref, d_ref, b1_ref, b2_ref, fm_ref, fi_ref,
               o_hbm,
               xT, xnT, hT, kT, vT, fT, sT, w1buf, w2buf, acc, uacc, ubf,
               kvb, Xs, Gs, Ys, taps, tpad, obuf,
               sem_q, sem_w10, sem_w1, sem_w2, sem_kvf, sem_o):

        def cp_q(i):
            cs = pl.ds(QB[i], QB[i + 1] - QB[i])
            return pltpu.make_async_copy(q_hbm.at[:, cs], xT.at[:, cs], sem_q.at[i])

        def cp_w10(i):
            ks = pl.ds(QB[i], QB[i + 1] - QB[i])
            return pltpu.make_async_copy(w1_hbm.at[ks, pl.ds(0, TF)], w1buf.at[0, ks, :], sem_w10.at[i])

        def cp_w1(t):
            return pltpu.make_async_copy(w1_hbm.at[:, pl.ds(pl.multiple_of(t * TF, TF), TF)], w1buf.at[t % 2], sem_w1.at[t % 2])

        def cp_w2(t):
            return pltpu.make_async_copy(w2_hbm.at[pl.ds(pl.multiple_of(t * TF, TF), TF), :], w2buf.at[t % 2], sem_w2.at[t % 2])

        def cp_kvf(c):
            rows = pl.ds(pl.multiple_of(c * CC, 8), CC)
            return [pltpu.make_async_copy(src.at[rows, :], dst.at[rows, :], sem_kvf.at[a, c % 2])
                    for a, (src, dst) in enumerate(((k_hbm, kT), (v_hbm, vT), (f_hbm, fT)))]

        def cp_o(i):
            cs = pl.ds(OB[i], OB[i + 1] - OB[i])
            return pltpu.make_async_copy(obuf.at[:, cs], o_hbm.at[:, cs], sem_o.at[i])

        for i in range(NQ):
            cp_q(i).start()
            cp_w10(i).start()

        tpad[...] = jnp.zeros_like(tpad)
        tpad[0:KS, 0:D] = sk_ref[...].astype(F32)
        tpad[KS:KS + 1, 0:D] = d_ref[...].astype(F32).reshape(1, D)
        for ct in range(5):
            taps[ct * 128:(ct + 1) * 128, :] = tpad[:, ct * 128:(ct + 1) * 128].T

        lane = lax.broadcasted_iota(jnp.int32, (8, 128), 1)
        sgn8 = (1 - 2 * (lane & 1)).astype(F32)

        zmask0 = jnp.full((8, 128), zs_ref[3], jnp.int32)

        def token(v, frac):
            r8 = min(v.shape[0] // 8 - 1, int(frac * (v.shape[0] // 8)))
            return pltpu.bitcast(v[r8 * 8:r8 * 8 + 8, 0:128], jnp.int32) & zmask0

        def gate16(x, tok):
            if tok is None:
                return x
            xi = pltpu.bitcast(x, jnp.int32)
            return pltpu.bitcast(xi | jnp.tile(tok, (xi.shape[0] // 8, 1)), BF)

        def ln_steps(lo, hi):
            for c0 in range(lo, hi, 128):
                cols = pl.ds(c0, 128)
                starts = range(0, D, LNB)

                def ldx(r, k, tok):
                    rows = pl.ds(r, LNB) if k is None else pl.ds(pl.multiple_of(r + zs_ref[k], 16), LNB)
                    return gate16(xT[rows, cols], tok).astype(F32)

                def fold(t, v):
                    for g in range(LNB // 8):
                        p_ = v[g * 8:(g + 1) * 8]
                        t = p_ if t is None else t + p_
                    return t

                t = None
                for r in starts:
                    tok = yield
                    t = fold(t, ldx(r, None, tok))
                m = jnp.sum(t, axis=0, keepdims=True) * (1.0 / D)
                t = None
                for r in starts:
                    tok = yield
                    xc = ldx(r, 0, tok) - m
                    t = fold(t, xc * xc)
                var = jnp.sum(t, axis=0, keepdims=True) * (1.0 / D)
                rs = lax.rsqrt(var + EPS)
                rsh = rs * lax.rsqrt(var * rs * rs + EPS)
                for r in starts:
                    tok = yield
                    xc = ldx(r, 1, tok) - m
                    xnT[pl.ds(r, LNB), cols] = (xc * rs).astype(BF)
                    hT[pl.ds(r, LNB), cols] = (xc * rsh).astype(BF)

        def ln_nsteps(lo, hi):
            return (hi - lo) // 128 * 3 * (D // LNB)

        def ln_run(lo, hi):
            gen = ln_steps(lo, hi)
            next(gen)
            for _ in range(ln_nsteps(lo, hi) - 1):
                gen.send(None)
            try:
                gen.send(None)
            except StopIteration:
                pass

        def b1_row(t):
            return b1_ref[pl.ds(pl.multiple_of(t * TF, TF), TF)].astype(F32).reshape(1, TF)

        def gate(x, tok):
            if tok is None:
                return x
            t = tok if x.shape[0] == 8 else jnp.tile(tok, (x.shape[0] // 8, 1))
            return pltpu.bitcast(pltpu.bitcast(x, jnp.int32) | t, F32)

        prep_state = {}

        def conv_prep(c0, j0, j1, tok):
            rows = pl.ds(pl.multiple_of(c0, 8), CC)
            tp = taps[rows, :]
            w = [jnp.broadcast_to(tp[:, tau:tau + 1], (CC, BL)) for tau in range(KS)]
            ln = lax.broadcasted_iota(jnp.int32, (CC, BL), 1)
            for j in range(j0, j1):
                cols = slice(j * BL, (j + 1) * BL)
                kb = gate(kT[rows, cols].astype(F32), tok)
                cur = [pltpu.roll(kb, tau, 1) for tau in range(1, KS)]
                ksh = kb * w[0]
                for tau in range(1, KS):
                    fill = 0.0 if j == 0 else prep_state["rolled"][tau - 1]
                    ksh = ksh + jnp.where(ln >= tau, cur[tau - 1], fill) * w[tau]
                prep_state["rolled"] = cur
                kvb[j * CC:(j + 1) * CC, :] = (ksh * vT[rows, cols].astype(F32)).astype(BF)

        def conv_dft_x():
            Xs[...] = _dot(kvb[...], fm_ref[...])

        def conv_dft_h(c0):
            rows = pl.ds(pl.multiple_of(c0, 8), CC)
            hb = jnp.concatenate([fT[rows, m * BL:(m + 1) * BL] for m in range(J)], axis=0)
            Gs[...] = _dot(hb, fm_ref[...])

        mac_state = {}

        def conv_mac(c0, r0, jb, tok=None):
            def ld(ref, j, o):
                return ref[j * CC + r0:j * CC + r0 + MR, o:o + BL]
            j0 = jb * JB
            sg = jnp.tile(sgn8, (MR // 8, 1))
            js = list(range(j0, j0 + JB))
            yr = {j: None for j in js}
            yi = {j: None for j in js}
            hwin = {}
            for i in range(js[-1], -1, -1):
                xr, xi = gate(ld(Xs, i, 0), tok), gate(ld(Xs, i, BL), tok)
                for j in js:
                    m = j - i
                    if m < 0:
                        continue
                    if m not in hwin:
                        hr = ld(Gs, m, 0)
                        if m == 0:
                            hr = hr + jnp.broadcast_to(taps[pl.ds(pl.multiple_of(c0 + r0, 8), MR), KS:KS + 1], (MR, BL))
                        hwin[m] = (hr, ld(Gs, m, BL))
                    hr, hi = hwin[m]
                    tr = xr * hr - xi * hi
                    ti = xr * hi + xi * hr
                    yr[j] = tr if yr[j] is None else yr[j] + tr
                    yi[j] = ti if yi[j] is None else yi[j] + ti
            for j in js:
                if j == 0:
                    zr, zi = yr[j], yi[j]
                else:
                    pyr, pyi = mac_state[r0]
                    zr = yr[j] - sg * pyi
                    zi = yi[j] + sg * pyr
                mac_state[r0] = (yr[j], yi[j])
                Ys[j * CC + r0:j * CC + r0 + MR, 0:BL] = zr.astype(Ys.dtype)
                Ys[j * CC + r0:j * CC + r0 + MR, BL:2 * BL] = zi.astype(Ys.dtype)

        def conv_inv(c0):
            rows = pl.ds(pl.multiple_of(c0, 8), CC)
            y = _dot(Ys[...].astype(BF), fi_ref[...])
            for j in range(J):
                cols = slice(j * BL, (j + 1) * BL)
                sT[rows, cols] = (xnT[rows, cols].astype(F32) * y[j * CC:(j + 1) * CC]).astype(BF)

        cp_q(0).wait()
        ln_run(QB[0], QB[1])
        b1r0 = b1_row(0)
        late = {1: [cp_w1(1)], 2: cp_kvf(0), 3: [cp_w2(0)]}
        for i in range(NQ):
            if i + 1 < NQ:
                cp_q(i + 1).wait()
            cp_w10(i).wait()
            for cp in late.get(i, []):
                cp.start()
            ks = slice(QB[i], QB[i + 1])
            hosts = list(range(TF // 128))
            if i + 1 < NQ:
                gen = ln_steps(QB[i + 1], QB[i + 2])
                next(gen)
                ns = ln_nsteps(QB[i + 1], QB[i + 2])
                plan = spread(list(range(ns)), [1] * ns, hosts)
            else:
                gen = None
                plan = [(h, []) for h in hosts]
            for n, cur in plan:
                cs = slice(n * 128, (n + 1) * 128)
                p = _dot(hT[:, ks], w1buf[0, ks, cs])
                for _, frac in cur:
                    try:
                        gen.send(token(p, frac))
                    except StopIteration:
                        pass
                if i == 0:
                    uacc[:, cs] = p
                elif i + 1 < NQ:
                    uacc[:, cs] += p
                else:
                    ubf[0, :, cs] = _gelu(uacc[:, cs] + p + b1r0[:, cs]).astype(BF)
            if i == NQ - 1:
                acc[...] = jnp.zeros_like(acc)

        def body(t, _):
            c = t - 1
            c0 = c * CC
            s1 = t % 2
            s2 = (t - 1) % 2

            cp_w1(t).wait()
            for cp in cp_kvf(c):
                cp.wait()

            def prefetch_a():
                @pl.when(t + 1 < NF)
                def _():
                    cp_w1(t + 1).start()
                    for cp in cp_kvf(c + 1):
                        cp.start()

            b1r = b1_row(t)
            conv_dft_h(c0)
            hosts = [(n, kq) for n in range(TF // N1) for kq in range(KQ)]
            nh = max(1, int(round(len(hosts) * PFRAC)))
            items = list(range(J // PJ))
            plan = spread(items, [1] * len(items), hosts[:nh]) + [(h, []) for h in hosts[nh:]]
            u = None
            kw = S // KQ
            for idx, ((n, kq), cur) in enumerate(plan):
                cs = slice(n * N1, (n + 1) * N1)
                p = _dot(hT[:, kq * kw:(kq + 1) * kw], w1buf[s1, kq * kw:(kq + 1) * kw, cs])
                for jq, frac in cur:
                    conv_prep(c0, jq * PJ, (jq + 1) * PJ, token(p, frac))
                u = p if kq == 0 else u + p
                if kq == KQ - 1:
                    ubf[s1, :, cs] = _gelu(u + b1r[:, cs]).astype(BF)
                if idx == nh - 1:
                    conv_dft_x()
                if idx == DMAPOS:
                    prefetch_a()

            cp_w2(t - 1).wait()

            hosts = list(range(S // N2))
            nh = max(1, int(round(len(hosts) * MFRAC)))
            items = [(g, jb) for g in range(CC // MR) for jb in range(J // JB)]
            cost = [jb * JB + JB for g, jb in items]
            plan = spread(items, cost, hosts[:nh]) + [(h, []) for h in hosts[nh:]]
            for idx, (n, cur) in enumerate(plan):
                cs = slice(n * N2, (n + 1) * N2)
                r = _dot(ubf[s2], w2buf[s2, :, cs])
                for (g, jb), frac in cur:
                    conv_mac(c0, g * MR, jb, token(r, frac))
                acc[:, cs] += r
                if idx == DMAPOS:
                    cp_w2(t).start()
                if idx == nh - 1:
                    conv_inv(c0)
            return None

        lax.fori_loop(1, NF, body, None)

        t = NF - 1
        cp_w2(t).wait()
        b2row = b2_ref[...].astype(F32).reshape(1, S)
        for n in range(NO):
            for c_ in range(OB[n], OB[n + 1], 128):
                cs = slice(c_, c_ + 128)
                y2 = acc[:, cs] + _dot(ubf[t % 2], w2buf[t % 2, :, cs]) + b2row[:, cs]
                g = (y2 * jax.nn.sigmoid(y2)).astype(BF).astype(F32)
                sg_ = sT[:, cs].astype(F32) * g
                obuf[:, cs] = (xT[:, cs].astype(F32) + sg_).astype(BF)
            cp_o(n).start()
        for n in range(NO):
            cp_o(n).wait()

    def run(A_q, A_k, A_v, A_shift_k, A_ssm_k, A_ssm_D, B_x, B_w1, B_b1, B_w2, B_b2):
        anyspec = pl.BlockSpec(memory_space=pl.ANY)
        vspec = pl.BlockSpec(memory_space=pltpu.VMEM)
        big = pltpu.VMEM((D, S), BF)
        out = pl.pallas_call(
            kernel,
            out_shape=jax.ShapeDtypeStruct((D, S), BF),
            in_specs=[pl.BlockSpec(memory_space=pltpu.SMEM)] + [anyspec] * 6 + [vspec] * 6,
            out_specs=anyspec,
            scratch_shapes=[
                big, big, big, big, big, big, big,
                pltpu.VMEM((2, S, TF), BF), pltpu.VMEM((2, TF, S), BF),
                pltpu.VMEM((D, S), F32), pltpu.VMEM((D, TF), F32), pltpu.VMEM((2, D, TF), BF),
                pltpu.VMEM((J * CC, BL), BF),
                pltpu.VMEM((J * CC, 2 * BL), F32), pltpu.VMEM((J * CC, 2 * BL), F32),
                pltpu.VMEM((J * CC, 2 * BL), F32),
                pltpu.VMEM((640, 128), F32), pltpu.VMEM((128, 640), F32),
                big,
                pltpu.SemaphoreType.DMA((NQ,)), pltpu.SemaphoreType.DMA((NQ,)),
                pltpu.SemaphoreType.DMA((2,)), pltpu.SemaphoreType.DMA((2,)),
                pltpu.SemaphoreType.DMA((3, 2)), pltpu.SemaphoreType.DMA((NO,)),
            ],
            compiler_params=pltpu.CompilerParams(vmem_limit_bytes=100 * 1024 * 1024),
        )(jnp.asarray(ZS_NP), A_q.reshape(S, D).T, A_k.reshape(S, D).T, A_v.reshape(S, D).T, A_ssm_k, B_w1, B_w2,
          A_shift_k.T, A_ssm_D, B_b1, B_b2, jnp.asarray(FM_NP), jnp.asarray(FI_NP))
        return out.T.reshape(1, S, D)

    return run


_run = _build()


@jax.jit
def pallas_recurrent_scan__ssm_conv_h3__mixer_token_mlp__prompt_kernel(
        A_q, A_k, A_v, A_shift_k, A_ssm_k, A_ssm_D, B_x, B_w1, B_b1, B_w2, B_b2):
    return _run(A_q, A_k, A_v, A_shift_k, A_ssm_k, A_ssm_D, B_x, B_w1, B_b1, B_w2, B_b2)
```
